```python
import os as _os
_os.environ.setdefault("JAX_PLATFORMS", "cpu")
import jax
import jax.numpy as jnp

def _softmax(x, axis=-1):
    return jax.nn.softmax(x, axis=axis)
def _gelu(x):
    return jax.nn.gelu(x, approximate=True)
def _silu(x):
    return jax.nn.silu(x)
def _sigmoid(x):
    return jax.nn.sigmoid(x)
def _layernorm(x, axis=-1, eps=1e-5):
    m = jnp.mean(x, axis=axis, keepdims=True)
    v = jnp.var(x, axis=axis, keepdims=True)
    return (x - m) / jnp.sqrt(v + eps)
def _scatter_add(tgt, idx, src, axis=0):
    return tgt.at[idx].add(src)
def _segment_sum(src, seg, n):
    return jax.ops.segment_sum(src, seg, n)
class _Rng:
    def __init__(self, key):
        self._k = key
    def _next(self):
        self._k, sub = jax.random.split(self._k)
        return sub
    def normal(self, shape):
        return jax.random.normal(self._next(), shape, dtype=jnp.bfloat16)
    def randint(self, lo, hi, shape):
        return jax.random.randint(self._next(), shape, lo, hi, dtype=jnp.int32)
    def uniform(self, shape, lo=0.0, hi=1.0):
        return jax.random.uniform(self._next(), shape, jnp.bfloat16, lo, hi)
    def permutation(self, n):
        return jax.random.permutation(self._next(), n)


kernel_name = 'standalone__gqa_softmax__near_ridge'

def setup_inputs():
    _rng = _Rng(jax.random.key(int.from_bytes(__import__("os").urandom(4), "little")))
    _w = (lambda a: (lambda t: t.astype(jnp.bfloat16) if jnp.issubdtype(t.dtype, jnp.floating) else t)(jnp.asarray(a)))
    B, Hq, Hkv, Sq, Sk, D = 8, 16, 8, 160, 2048, 256
    return {
        "q": _w((lambda *s: _rng.normal(s) * 0.05)(B, Hq, Sq, D)),
        "k": _w((lambda *s: _rng.normal(s) * 3.2)(B, Hkv, Sk, D)),
        "v": _w((lambda *s: _rng.normal(s) * 0.05)(B, Hkv, Sk, D)),
    }

def reference(q, k, v):
    B, Hq, Sq, D = q.shape
    Hkv = k.shape[1]
    rep = Hq // Hkv
    k = jnp.repeat(k, rep, axis=1)
    v = jnp.repeat(v, rep, axis=1)
    scale = D ** -0.5
    scores = jnp.einsum("bhqd,bhkd->bhqk", q, k) * scale
    p = _softmax(scores, axis=-1)
    return jnp.einsum("bhqk,bhkd->bhqd", p, v)
```

```python
import functools

import jax
import jax.numpy as jnp
import jax.experimental.pallas as pl
import jax.experimental.pallas.tpu as pltpu

_LOG2E = 1.4426950408889634


def _attn_kernel(q_ref, k_ref, v_ref, o_ref, *, scale):
    q = q_ref[0]
    k = k_ref[0]
    v = v_ref[0]
    s = jax.lax.dot_general(q, k, (((1,), (1,)), ((), ())), preferred_element_type=jnp.float32)
    m = jnp.max(s, axis=-1, keepdims=True)
    p = jnp.exp2((s - m) * (scale * _LOG2E))
    l = jnp.sum(p, axis=-1, keepdims=True)
    o = jnp.dot(p.astype(jnp.bfloat16), v, preferred_element_type=jnp.float32)
    o_ref[0] = (o / l).astype(o_ref.dtype)


@jax.jit
def pallas_standalone__gqa_softmax__near_ridge_kernel(q, k, v):
    B, Hq, Sq, D = q.shape
    Hkv, Sk = k.shape[1], k.shape[2]
    rep = Hq // Hkv
    G = B * Hkv
    M = rep * Sq
    q3 = q.reshape(G, M, D)
    k3 = k.reshape(G, Sk, D)
    v3 = v.reshape(G, Sk, D)
    out = pl.pallas_call(
        functools.partial(_attn_kernel, scale=D ** -0.5),
        grid=(G,),
        in_specs=[
            pl.BlockSpec((1, M, D), lambda g: (g, 0, 0)),
            pl.BlockSpec((1, Sk, D), lambda g: (g, 0, 0)),
            pl.BlockSpec((1, Sk, D), lambda g: (g, 0, 0)),
        ],
        out_specs=pl.BlockSpec((1, M, D), lambda g: (g, 0, 0)),
        out_shape=jax.ShapeDtypeStruct((G, M, D), q.dtype),
        compiler_params=pltpu.CompilerParams(
            dimension_semantics=("parallel",),
            vmem_limit_bytes=64 * 1024 * 1024,
        ),
    )(q3, k3, v3)
    return out.reshape(B, Hq, Sq, D)
```

```python
import functools

import jax
import jax.numpy as jnp
from jax import lax
import jax.experimental.pallas as pl
import jax.experimental.pallas.tpu as pltpu

_LOG2E = 1.4426950408889634
_NT = (((1,), (1,)), ((), ()))
_LANES = 128

_UNROLL = 9
_NCHUNK = 2
_DOT_KEYS = 256
_NSCORE = 3


def _attention_kernel(q_hbm, k_hbm, v_hbm, o_hbm,
                      q_buf, k_buf, v_buf, o_buf, s_buf, m_buf, sem, *, scale):
    n_heads, rows, _ = q_hbm.shape
    n_keys = k_hbm.shape[1]
    unroll, nchunk, dk = _UNROLL, _NCHUNK, _DOT_KEYS
    ck = n_keys // nchunk
    ring = unroll * nchunk
    n_chunks = n_heads * nchunk
    n_pieces = n_keys // dk
    c_exp2 = scale * _LOG2E
    sem_q, sem_k, sem_v, sem_o = 0, unroll, unroll + ring, unroll + 2 * ring
    sem_first = 2 * unroll + 2 * ring

    def q_copy(h, slot):
        return pltpu.make_async_copy(q_hbm.at[h], q_buf.at[slot], sem.at[sem_q + slot])

    def k_copy(j, slot):
        src = k_hbm.at[j // nchunk, pl.ds(lax.rem(j, nchunk) * ck, ck)]
        return pltpu.make_async_copy(src, k_buf.at[slot], sem.at[sem_k + slot])

    def v_copy(j, slot):
        src = v_hbm.at[j // nchunk, pl.ds(lax.rem(j, nchunk) * ck, ck)]
        return pltpu.make_async_copy(src, v_buf.at[slot], sem.at[sem_v + slot])

    def o_copy(h, slot):
        return pltpu.make_async_copy(o_buf.at[slot], o_hbm.at[h], sem.at[sem_o + slot])

    def first_k_copy(p):
        slot, off = divmod(p * dk, ck)
        return pltpu.make_async_copy(k_hbm.at[0, pl.ds(p * dk, dk)],
                                     k_buf.at[slot, pl.ds(off, dk)],
                                     sem.at[sem_first + p])

    def when(cond, fn):
        if isinstance(cond, bool):
            if cond:
                fn()
        else:
            pl.when(cond)(fn)

    def stage(t, phase, zero, do_qk, do_pv, finish_prev=None, defer=False):
        qk_slot, pv_slot = (phase + 1) % unroll, phase % unroll
        s_old = s_buf.at[phase % _NSCORE + zero]
        s_new = s_buf.at[(phase + 1) % _NSCORE + zero]
        m_old = m_buf.at[phase % _NSCORE + zero]
        m_new = m_buf.at[(phase + 1) % _NSCORE + zero]
        q = row_max = col_max = col_sum = acc = None

        for c in range(nchunk):
            g = (t + 1) * nchunk + c
            k_slot, v_slot = qk_slot * nchunk + c, pv_slot * nchunk + c

            if do_qk and do_pv:
                if c == 0:
                    q_copy(t + 1, qk_slot).wait()
                k_copy(g, k_slot).wait()
            if c == 0 and finish_prev is not None:
                finish_prev()

            if do_qk:
                for b in range(0, ck, dk):
                    if not do_pv:
                        first_k_copy((c * ck + b) // dk).wait()
                    k = k_buf[k_slot, b:b + dk, :]
                    if q is None:
                        q = q_buf[qk_slot]
                    s = lax.dot_general(q, k, _NT, preferred_element_type=jnp.float32)
                    s_new[:, c * ck + b:c * ck + b + dk] = s
                    tile_max = s[:, :_LANES]
                    for j in range(_LANES, dk, _LANES):
                        tile_max = jnp.maximum(tile_max, s[:, j:j + _LANES])
                    col_max = tile_max if col_max is None else jnp.maximum(col_max, tile_max)

            if c == 0:
                when(t >= 1, lambda: o_copy(t - 1, (pv_slot - 1) % unroll).start())
            if do_pv:
                v_copy(g - nchunk, v_slot).wait()
                if c == nchunk - 1:
                    when(t >= unroll, lambda: o_copy(t - unroll, pv_slot).wait())
            gv = g - nchunk - 1
            when((gv >= 0) & (gv + ring < n_chunks),
                 lambda: v_copy(gv + ring, (v_slot - 1) % ring).start())
            if c == 0:
                when(t + 1 + unroll < n_heads,
                     lambda: q_copy(t + 1 + unroll, qk_slot).start())
            when(g + ring < n_chunks, lambda: k_copy(g + ring, k_slot).start())

            if do_pv:
                for b in range(0, ck, dk):
                    if row_max is None:
                        row_max = m_old[...]
                    tiles = []
                    for j in range(0, dk, _LANES):
                        col = c * ck + b + j
                        p = jnp.exp2((s_old[:, col:col + _LANES] - row_max) * c_exp2)
                        col_sum = p if col_sum is None else col_sum + p
                        tiles.append(p.astype(jnp.bfloat16))
                    pv = jnp.dot(jnp.concatenate(tiles, axis=1), v_buf[v_slot, b:b + dk, :],
                                 preferred_element_type=jnp.float32)
                    acc = pv if acc is None else acc + pv

        if do_qk:
            m_new[...] = jnp.broadcast_to(jnp.max(col_max, axis=-1, keepdims=True), m_new.shape)
        if not do_pv:
            return None

        def finish():
            inv = 1.0 / jnp.sum(col_sum, axis=-1, keepdims=True)
            o_buf[pv_slot] = (acc * inv).astype(o_buf.dtype)

        if defer:
            return finish
        finish()
        return None

    first_k_copy(0).start()
    q_copy(0, 0).start()
    for p in range(1, n_pieces):
        first_k_copy(p).start()
    for h in range(1, unroll):
        q_copy(h, h).start()
        for c in range(nchunk):
            k_copy(h * nchunk + c, h * nchunk + c).start()
            v_copy((h - 1) * nchunk + c, (h - 1) * nchunk + c).start()
    for c in range(nchunk):
        v_copy((unroll - 1) * nchunk + c, (unroll - 1) * nchunk + c).start()

    q_copy(0, 0).wait()
    stage(-1, -1, 0, True, False)

    def body(i, _):
        zero = lax.rem(i * 2, 2)
        finish = None
        for u in range(unroll):
            finish = stage(i * unroll + u, u, zero, True, True, finish, u < unroll - 1)

    lax.fori_loop(0, (n_heads - 1) // unroll, body, None)

    last = n_heads - 1
    stage(last, last, 0, False, True)
    o_copy(last, last % unroll).start()
    for h in range(n_heads - unroll, n_heads):
        o_copy(h, h % unroll).wait()


@jax.jit
def pallas_standalone__gqa_softmax__near_ridge_kernel(
    q: jax.Array,
    k: jax.Array,
    v: jax.Array,
):
    batch, q_heads, q_len, d = q.shape
    kv_heads, k_len = k.shape[1], k.shape[2]
    n_heads = batch * kv_heads
    rows = (q_heads // kv_heads) * q_len
    ck = k_len // _NCHUNK
    ring = _UNROLL * _NCHUNK
    assert (n_heads - 1) % _UNROLL == 0 and _UNROLL % _NSCORE == 0
    assert k_len % (_NCHUNK * _DOT_KEYS) == 0

    hbm = pl.BlockSpec(memory_space=pl.ANY)
    out = pl.pallas_call(
        functools.partial(_attention_kernel, scale=d ** -0.5),
        in_specs=[hbm, hbm, hbm],
        out_specs=hbm,
        out_shape=jax.ShapeDtypeStruct((n_heads, rows, d), q.dtype),
        scratch_shapes=[
            pltpu.VMEM((_UNROLL, rows, d), q.dtype),
            pltpu.VMEM((ring, ck, d), k.dtype),
            pltpu.VMEM((ring, ck, d), v.dtype),
            pltpu.VMEM((_UNROLL, rows, d), q.dtype),
            pltpu.VMEM((_NSCORE, rows, k_len), jnp.float32),
            pltpu.VMEM((_NSCORE, rows, _LANES), jnp.float32),
            pltpu.SemaphoreType.DMA((2 * _UNROLL + 2 * ring + k_len // _DOT_KEYS,)),
        ],
        compiler_params=pltpu.CompilerParams(
            vmem_limit_bytes=64 * 1024 * 1024,
            disable_bounds_checks=True,
            disable_semaphore_checks=True,
            flags={"XLA_TPU_RESCHEDULE_DMA_DONES": True},
        ),
    )(
        q.reshape(n_heads, rows, d),
        k.reshape(n_heads, k_len, d),
        v.reshape(n_heads, k_len, d),
    )
    return out.reshape(batch, q_heads, q_len, d)
```

```python
import functools

import jax
import jax.numpy as jnp
from jax import lax
import jax.experimental.pallas as pl
import jax.experimental.pallas.tpu as pltpu

_LOG2E = 1.4426950408889634
_NT = (((1,), (1,)), ((), ()))
_LANES = 128

_UNROLL = 9
_NCHUNK = 2
_DOT_KEYS = 256
_NSCORE = 3
_TAIL_SPLIT = 4


def _attention_kernel(q_hbm, k_hbm, v_hbm, o_hbm,
                      q_buf, k_buf, v_buf, o_buf, s_buf, m_buf, sem, *, scale):
    n_heads, rows, _ = q_hbm.shape
    n_keys = k_hbm.shape[1]
    unroll, nchunk, dk = _UNROLL, _NCHUNK, _DOT_KEYS
    ck = n_keys // nchunk
    ring = unroll * nchunk
    n_chunks = n_heads * nchunk
    n_pieces = n_keys // dk
    c_exp2 = scale * _LOG2E
    sem_q, sem_k, sem_v, sem_o = 0, unroll, unroll + ring, unroll + 2 * ring
    sem_first = 2 * unroll + 2 * ring

    def q_copy(h, slot):
        return pltpu.make_async_copy(q_hbm.at[h], q_buf.at[slot], sem.at[sem_q + slot])

    def k_copy(j, slot):
        src = k_hbm.at[j // nchunk, pl.ds(lax.rem(j, nchunk) * ck, ck)]
        return pltpu.make_async_copy(src, k_buf.at[slot], sem.at[sem_k + slot])

    def v_copy(j, slot):
        src = v_hbm.at[j // nchunk, pl.ds(lax.rem(j, nchunk) * ck, ck)]
        return pltpu.make_async_copy(src, v_buf.at[slot], sem.at[sem_v + slot])

    def o_copy(h, slot):
        return pltpu.make_async_copy(o_buf.at[slot], o_hbm.at[h], sem.at[sem_o + slot])

    def first_k_copy(p):
        slot, off = divmod(p * dk, ck)
        return pltpu.make_async_copy(k_hbm.at[0, pl.ds(p * dk, dk)],
                                     k_buf.at[slot, pl.ds(off, dk)],
                                     sem.at[sem_first + p])

    def when(cond, fn):
        if isinstance(cond, bool):
            if cond:
                fn()
        else:
            pl.when(cond)(fn)

    def softmax_pv(s_ref, rs, col0, row_max, v_slot, b, col_sum, acc):
        tiles = []
        for col in range(col0, col0 + dk, _LANES):
            p = jnp.exp2((s_ref[rs, col:col + _LANES] - row_max) * c_exp2)
            col_sum = p if col_sum is None else col_sum + p
            tiles.append(p.astype(v_buf.dtype))
        pv = jnp.dot(jnp.concatenate(tiles, axis=1), v_buf[v_slot, b:b + dk, :],
                     preferred_element_type=jnp.float32)
        return col_sum, (pv if acc is None else acc + pv)

    def normalize(col_sum, acc):
        inv = 1.0 / jnp.sum(col_sum, axis=-1, keepdims=True)
        return (acc * inv).astype(o_buf.dtype)

    def stage(t, phase, zero, do_pv, finish_prev=None, defer=False):
        qk_slot, pv_slot = (phase + 1) % unroll, phase % unroll
        s_old = s_buf.at[phase % _NSCORE + zero]
        s_new = s_buf.at[(phase + 1) % _NSCORE + zero]
        m_old = m_buf.at[phase % _NSCORE + zero]
        m_new = m_buf.at[(phase + 1) % _NSCORE + zero]
        q = row_max = col_max = col_sum = acc = None

        for c in range(nchunk):
            g = (t + 1) * nchunk + c
            k_slot, v_slot = qk_slot * nchunk + c, pv_slot * nchunk + c

            if do_pv:
                if c == 0:
                    q_copy(t + 1, qk_slot).wait()
                k_copy(g, k_slot).wait()
            if c == 0 and finish_prev is not None:
                finish_prev()

            for b in range(0, ck, dk):
                if not do_pv:
                    first_k_copy((c * ck + b) // dk).wait()
                k = k_buf[k_slot, b:b + dk, :]
                if q is None:
                    q = q_buf[qk_slot]
                s = lax.dot_general(q, k, _NT, preferred_element_type=jnp.float32)
                s_new[:, c * ck + b:c * ck + b + dk] = s
                tile_max = s[:, :_LANES]
                for j in range(_LANES, dk, _LANES):
                    tile_max = jnp.maximum(tile_max, s[:, j:j + _LANES])
                col_max = tile_max if col_max is None else jnp.maximum(col_max, tile_max)

            if c == 0:
                when(t >= 1, lambda: o_copy(t - 1, (pv_slot - 1) % unroll).start())
            if do_pv:
                v_copy(g - nchunk, v_slot).wait()
                if c == nchunk - 1:
                    when(t >= unroll, lambda: o_copy(t - unroll, pv_slot).wait())
            gv = g - nchunk - 1
            when((gv >= 0) & (gv + ring < n_chunks),
                 lambda: v_copy(gv + ring, (v_slot - 1) % ring).start())
            if c == 0:
                when(t + 1 + unroll < n_heads,
                     lambda: q_copy(t + 1 + unroll, qk_slot).start())
            when(g + ring < n_chunks, lambda: k_copy(g + ring, k_slot).start())

            if do_pv:
                for b in range(0, ck, dk):
                    if row_max is None:
                        row_max = m_old[...]
                    col_sum, acc = softmax_pv(s_old, slice(None), c * ck + b, row_max,
                                              v_slot, b, col_sum, acc)

        m_new[...] = jnp.broadcast_to(jnp.max(col_max, axis=-1, keepdims=True), m_new.shape)
        if not do_pv:
            return None

        def finish():
            o_buf[pv_slot] = normalize(col_sum, acc)

        if defer:
            return finish
        finish()
        return None

    first_k_copy(0).start()
    q_copy(0, 0).start()
    for p in range(1, n_pieces):
        first_k_copy(p).start()
    for h in range(1, unroll):
        q_copy(h, h).start()
        for c in range(nchunk):
            k_copy(h * nchunk + c, h * nchunk + c).start()
            v_copy((h - 1) * nchunk + c, (h - 1) * nchunk + c).start()
    for c in range(nchunk):
        v_copy((unroll - 1) * nchunk + c, (unroll - 1) * nchunk + c).start()

    q_copy(0, 0).wait()
    stage(-1, -1, 0, False)

    def body(i, _):
        zero = lax.rem(i * 2, 2)
        finish = None
        for u in range(unroll):
            finish = stage(i * unroll + u, u, zero, True, finish, u < unroll - 1)

    lax.fori_loop(0, (n_heads - 1) // unroll, body, None)

    last = n_heads - 1
    slot, score = last % unroll, last % _NSCORE
    tail = rows // _TAIL_SPLIT

    def tail_copy(p):
        return pltpu.make_async_copy(o_buf.at[slot, pl.ds(p * tail, tail)],
                                     o_hbm.at[last, pl.ds(p * tail, tail)],
                                     sem.at[sem_first + p])

    o_copy(last - 1, (last - 1) % unroll).start()
    for c in range(nchunk):
        v_copy(last * nchunk + c, slot * nchunk + c).wait()
    o_copy(last - unroll, slot).wait()
    for p in range(_TAIL_SPLIT):
        rs = slice(p * tail, (p + 1) * tail)
        row_max = m_buf[score, rs, :]
        col_sum = acc = None
        for col in range(0, n_keys, dk):
            col_sum, acc = softmax_pv(s_buf.at[score], rs, col, row_max,
                                      slot * nchunk + col // ck, col % ck, col_sum, acc)
        o_buf[slot, rs, :] = normalize(col_sum, acc)
        tail_copy(p).start()
    for h in range(n_heads - unroll, last):
        o_copy(h, h % unroll).wait()
    for p in range(_TAIL_SPLIT):
        tail_copy(p).wait()


@jax.jit
def pallas_standalone__gqa_softmax__near_ridge_kernel(
    q: jax.Array,
    k: jax.Array,
    v: jax.Array,
):
    batch, q_heads, q_len, d = q.shape
    kv_heads, k_len = k.shape[1], k.shape[2]
    n_heads = batch * kv_heads
    rows = (q_heads // kv_heads) * q_len
    ck = k_len // _NCHUNK
    ring = _UNROLL * _NCHUNK
    assert (n_heads - 1) % _UNROLL == 0 and _UNROLL % _NSCORE == 0
    assert k_len % (_NCHUNK * _DOT_KEYS) == 0
    assert rows % (16 * _TAIL_SPLIT) == 0 and _TAIL_SPLIT <= k_len // _DOT_KEYS

    hbm = pl.BlockSpec(memory_space=pl.ANY)
    out = pl.pallas_call(
        functools.partial(_attention_kernel, scale=d ** -0.5),
        in_specs=[hbm, hbm, hbm],
        out_specs=hbm,
        out_shape=jax.ShapeDtypeStruct((n_heads, rows, d), q.dtype),
        scratch_shapes=[
            pltpu.VMEM((_UNROLL, rows, d), q.dtype),
            pltpu.VMEM((ring, ck, d), k.dtype),
            pltpu.VMEM((ring, ck, d), v.dtype),
            pltpu.VMEM((_UNROLL, rows, d), q.dtype),
            pltpu.VMEM((_NSCORE, rows, k_len), jnp.float32),
            pltpu.VMEM((_NSCORE, rows, _LANES), jnp.float32),
            pltpu.SemaphoreType.DMA((2 * _UNROLL + 2 * ring + k_len // _DOT_KEYS,)),
        ],
        compiler_params=pltpu.CompilerParams(
            vmem_limit_bytes=64 * 1024 * 1024,
            disable_bounds_checks=True,
            disable_semaphore_checks=True,
            flags={"XLA_TPU_RESCHEDULE_DMA_DONES": True},
        ),
    )(
        q.reshape(n_heads, rows, d),
        k.reshape(n_heads, k_len, d),
        v.reshape(n_heads, k_len, d),
    )
    return out.reshape(batch, q_heads, q_len, d)
```
